```python
import os as _os
_os.environ.setdefault("JAX_PLATFORMS", "cpu")
import jax
import jax.numpy as jnp

def _softmax(x, axis=-1):
    return jax.nn.softmax(x, axis=axis)
def _gelu(x):
    return jax.nn.gelu(x, approximate=True)
def _silu(x):
    return jax.nn.silu(x)
def _sigmoid(x):
    return jax.nn.sigmoid(x)
def _layernorm(x, axis=-1, eps=1e-5):
    m = jnp.mean(x, axis=axis, keepdims=True)
    v = jnp.var(x, axis=axis, keepdims=True)
    return (x - m) / jnp.sqrt(v + eps)
def _scatter_add(tgt, idx, src, axis=0):
    return tgt.at[idx].add(src)
def _segment_sum(src, seg, n):
    return jax.ops.segment_sum(src, seg, n)
class _Rng:
    def __init__(self, key):
        self._k = key
    def _next(self):
        self._k, sub = jax.random.split(self._k)
        return sub
    def normal(self, shape):
        return jax.random.normal(self._next(), shape, dtype=jnp.bfloat16)
    def randint(self, lo, hi, shape):
        return jax.random.randint(self._next(), shape, lo, hi, dtype=jnp.int32)
    def uniform(self, shape, lo=0.0, hi=1.0):
        return jax.random.uniform(self._next(), shape, jnp.bfloat16, lo, hi)
    def permutation(self, n):
        return jax.random.permutation(self._next(), n)


kernel_name = 'parallel_sum__sliding_block__moe_arch_mod__prompt'

def setup_inputs():
    _rng = _Rng(jax.random.key(int.from_bytes(__import__("os").urandom(4), "little")))
    _w = (lambda a: (lambda t: t.astype(jnp.bfloat16) if jnp.issubdtype(t.dtype, jnp.floating) else t)(jnp.asarray(a)))
    def _A_setup():
        B, S, D = 1, 2048, 512
        return {
            "x": _w((lambda *s: _rng.normal(s) * 0.05)(B, S, D)),
            "wqkv": _w((lambda *s: _rng.normal(s) * 0.05)(D, 3 * D)),
            "wo": _w((lambda *s: _rng.normal(s) * 0.05)(D, D)),
        }
    _A_in = _A_setup()

    def _B_setup():
        B, S, D, F, C = 1, 2048, 512, 1376, 1
        return {
            "x": _w((lambda *s: _rng.normal(s) * 0.05)(B, S, D)),
            "w_r": _w((lambda *s: _rng.normal(s) * 0.05)(D)),
            "w_gate": _w((lambda *s: _rng.normal(s) * 0.05)(D, F)),
            "w_up": _w((lambda *s: _rng.normal(s) * 0.05)(D, F)),
            "w_down": _w((lambda *s: _rng.normal(s) * 0.05)(F, D)),
        }
    _B_in = _B_setup()

    return {
        "A_x": _A_in["x"],
        "A_wqkv": _A_in["wqkv"],
        "A_wo": _A_in["wo"],
        "B_x": _B_in["x"],
        "B_w_r": _B_in["w_r"],
        "B_w_gate": _B_in["w_gate"],
        "B_w_up": _B_in["w_up"],
        "B_w_down": _B_in["w_down"],
    }

def reference(A_x, A_wqkv, A_wo, B_x, B_w_r, B_w_gate, B_w_up, B_w_down):
    def _A_ref(x, wqkv, wo):
        B, S, D = x.shape
        H = 32; Dh = D // H; W = 256
        qkv = (lambda x, *d: x.transpose(*d))((x @ wqkv).reshape(B, S, 3, H, Dh), 2, 0, 3, 1, 4)
        q, k, v = qkv[0], qkv[1], qkv[2]
        scores = jnp.einsum("bhqd,bhkd->bhqk", q, k) * (Dh ** -0.5)
        idx = jnp.arange(S)
        mask = (idx[:, None] - idx[None, :] >= 0) & (idx[:, None] - idx[None, :] < W)
        scores = jnp.where(mask[None, None], scores, -1e9)
        p = _softmax(scores, axis=-1)
        o = jnp.einsum("bhqk,bhkd->bhqd", p, v)
        return (lambda x, *d: x.transpose(*d))(o, 0, 2, 1, 3).reshape(B, S, D) @ wo

    def _B_ref(x, w_r, w_gate, w_up, w_down):
        B, S, D = x.shape
        C = 1
        r = x @ w_r
        idx = jnp.argsort(-r, axis=-1)[:, :C]
        idx_e = jnp.repeat(idx.reshape(B, C, 1), D, axis=2)
        x_sel = jnp.take_along_axis(x, idx_e, axis=1)
        g = _silu(x_sel @ w_gate)
        u = x_sel @ w_up
        y = (g * u) @ w_down
        r_sel = _sigmoid(jnp.take_along_axis(r, idx, axis=1))
        y = y * r_sel.reshape(B, C, 1)
        b_off = (jnp.arange(B) * S).reshape(B, 1)
        flat_idx = (idx + b_off).reshape(B * C)
        zero = (x * 0.0).reshape(B * S, D)
        upd = _scatter_add(zero, flat_idx, y.reshape(B * C, D), axis=0)
        return x + upd.reshape(B, S, D)

    x = A_x
    xn = _layernorm(x, axis=-1)
    return x + _A_ref(xn, A_wqkv, A_wo) + _B_ref(xn, B_w_r, B_w_gate, B_w_up, B_w_down)
```

```python
import jax
import jax.numpy as jnp
import jax.experimental.pallas as pl
import jax.experimental.pallas.tpu as pltpu

S = 2048
D = 512
H = 32
DH = 16
W = 256
F = 1376
NEG = -1e9
LOG2E = 1.4426950408889634
QSCALE = (DH ** -0.5) * LOG2E
R = 256
NCH = S // R
QB = 128
M = S // QB
PAD = 256

_NT = (((1,), (1,)), ((), ()))


def _bf(a):
    return a.astype(jnp.bfloat16).astype(jnp.float32)


def _kernel(x_hbm, wqkv_hbm, wo_hbm, wr_ref, wg_hbm, wu_hbm, wd_hbm, out_hbm,
            x_v, xn_v, wqkv_v, wvt_v, wo_v, q_v, k_v, vt_v, r_v,
            s_buf0, s_buf1, mx_buf0, mx_buf1, ot0, ot1,
            wg_v, wu_v, wd_v, moe_v, idx_v,
            x_sems, w_sems, o_sem):
    f32 = jnp.float32
    bf16 = jnp.bfloat16
    s_bufs = (s_buf0, s_buf1)
    mx_bufs = (mx_buf0, mx_buf1)
    ots = (ot0, ot1)

    def x_copy(c):
        return pltpu.make_async_copy(x_hbm.at[pl.ds(c * R, R)], x_v.at[pl.ds(c * R, R)], x_sems.at[c])

    w_copies = [
        pltpu.make_async_copy(wqkv_hbm, wqkv_v, w_sems.at[0]),
        pltpu.make_async_copy(wo_hbm, wo_v, w_sems.at[1]),
        pltpu.make_async_copy(wg_hbm, wg_v, w_sems.at[2]),
        pltpu.make_async_copy(wu_hbm, wu_v, w_sems.at[3]),
        pltpu.make_async_copy(wd_hbm, wd_v, w_sems.at[4]),
    ]
    x_copy(0).start()
    w_copies[0].start()
    for c in range(1, NCH):
        x_copy(c).start()
    for cp in w_copies[1:]:
        cp.start()

    k_v[0:PAD, :] = jnp.zeros((PAD, D), bf16)
    vt_v[:, 0:PAD] = jnp.zeros((D, PAD), bf16)

    w_copies[0].wait()
    wvt_v[...] = wqkv_v[:, 2 * D:3 * D].astype(f32).T.astype(bf16)

    wr = wr_ref[...].astype(f32)

    def phase0(c, carry):
        r0 = pl.multiple_of(c * R, R)
        x_copy(c).wait()
        xf = x_v[pl.ds(r0, R), :].astype(f32)
        mean = jnp.mean(xf, axis=-1, keepdims=True)
        var = jnp.mean(jnp.square(xf - mean), axis=-1, keepdims=True)
        dlt = _bf(xf - _bf(mean))
        den = _bf(jnp.sqrt(_bf(_bf(var) + 1e-5)))
        xn = (dlt / den).astype(bf16)
        xn_v[pl.ds(r0, R), :] = xn
        r_v[pl.ds(r0, R), :] = _bf(jnp.sum(xn.astype(f32) * wr, axis=-1, keepdims=True))
        qk = jnp.dot(xn, wqkv_v[:, 0:2 * D], preferred_element_type=f32)
        q_v[pl.ds(r0, R), :] = (qk[:, 0:D] * QSCALE).astype(bf16)
        k_v[pl.ds(PAD + r0, R), :] = qk[:, D:2 * D].astype(bf16)
        vt = jax.lax.dot_general(wvt_v[...], xn, _NT, preferred_element_type=f32)
        vt_v[:, pl.ds(PAD + r0, R)] = vt.astype(bf16)
        return carry

    jax.lax.fori_loop(0, NCH, phase0, 0)

    rr = r_v[...]
    rmax = jnp.max(rr, axis=0, keepdims=True)
    ids = jax.lax.broadcasted_iota(jnp.int32, (S, 1), 0)
    idx = jnp.min(jnp.where(rr == rmax, ids, S), axis=0, keepdims=True)
    idx_v[...] = idx

    def gather_row(c, acc):
        r0 = pl.multiple_of(c * R, R)
        rows = jax.lax.broadcasted_iota(jnp.int32, (R, D), 0) + r0
        xc = xn_v[pl.ds(r0, R), :].astype(f32)
        return acc + jnp.sum(jnp.where(rows == idx, xc, 0.0), axis=0, keepdims=True)

    x_sel = jax.lax.fori_loop(0, NCH, gather_row, jnp.zeros((1, D), f32))
    xs16 = jnp.broadcast_to(x_sel, (16, D)).astype(bf16)
    for cp in w_copies[2:]:
        cp.wait()
    gate = jnp.dot(xs16, wg_v[...], preferred_element_type=f32)
    up = jnp.dot(xs16, wu_v[...], preferred_element_type=f32)
    hmid = (gate * jax.nn.sigmoid(gate) * up).astype(bf16)
    y = jnp.dot(hmid, wd_v[...], preferred_element_type=f32)
    moe_v[...] = y[0:1, :] * jax.nn.sigmoid(rmax)

    lane = jax.lax.broadcasted_iota(jnp.int32, (QB, QB), 1)
    row = jax.lax.broadcasted_iota(jnp.int32, (QB, QB), 0)
    lane_head = lane // DH
    tri = row <= lane

    def stage_a(m, g, slot, masked):
        q0 = pl.multiple_of(m * QB, QB)
        gl = slice(g * 128, (g + 1) * 128)
        qs = q_v[pl.ds(q0, QB), gl]
        kf = k_v[pl.ds(q0, QB), gl]
        km = k_v[pl.ds(q0 + QB, QB), gl]
        kd = k_v[pl.ds(q0 + 2 * QB, QB), gl]
        parts = []
        for r in range(8):
            parts.append(kf[16 * r:16 * r + 16])
            parts.append(kd[16 * r:16 * r + 16])
        parts.append(km)
        ks = jnp.concatenate(parts, axis=0)
        qstack = jnp.concatenate(
            [jnp.where(lane_head == h, qs, jnp.zeros_like(qs)) for h in range(8)], axis=0)
        st = jax.lax.dot_general(ks, qstack, _NT, preferred_element_type=f32)
        for h in range(8):
            sl = slice(h * 128, (h + 1) * 128)
            mparts = []
            for r in range(8):
                far = st[32 * r:32 * r + 16, sl]
                diag = st[32 * r + 16:32 * r + 32, sl]
                if masked:
                    far = jnp.where(m >= 2, far, NEG)
                mparts.append(jnp.where(tri[16 * r:16 * r + 16], diag, far))
            mid = st[256:384, sl]
            if masked:
                mid = jnp.where(m >= 1, mid, NEG)
            sm = jnp.concatenate(mparts, axis=0)
            mx = jnp.maximum(jnp.max(sm, axis=0, keepdims=True), jnp.max(mid, axis=0, keepdims=True))
            s_bufs[slot][0:128, sl] = sm
            s_bufs[slot][128:256, sl] = mid
            mx_bufs[slot][:, sl] = mx

    def stage_bc(m, g, slot, oslot):
        q0 = pl.multiple_of(m * QB, QB)
        for h in range(8):
            sl = slice(h * 128, (h + 1) * 128)
            hh = g * 8 + h
            mx = mx_bufs[slot][:, sl]
            p_m = jnp.exp2(s_bufs[slot][0:128, sl] - mx)
            p_mid = jnp.exp2(s_bufs[slot][128:256, sl] - mx)
            l = jnp.sum(p_m, axis=0, keepdims=True) + jnp.sum(p_mid, axis=0, keepdims=True)
            zero = jnp.zeros_like(p_m)
            p = jnp.concatenate([jnp.where(tri, zero, p_m), p_mid, jnp.where(tri, p_m, zero)],
                                axis=0).astype(bf16)
            vt = vt_v[16 * hh:16 * hh + 16, pl.ds(q0, 3 * QB)]
            ot = jnp.dot(vt, p, preferred_element_type=f32)
            ots[oslot][16 * hh:16 * hh + 16, :] = ot / l

    def stage_d(m, oslot):
        q0 = pl.multiple_of(m * QB, QB)
        o = ots[oslot][...].T.astype(bf16)
        att = jnp.dot(o, wo_v[...], preferred_element_type=f32)
        rows = jax.lax.broadcasted_iota(jnp.int32, (QB, D), 0) + q0
        res = x_v[pl.ds(q0, QB), :].astype(f32) + xn_v[pl.ds(q0, QB), :].astype(f32) + att
        res = res + jnp.where(rows == idx_v[...], moe_v[...], 0.0)
        x_v[pl.ds(q0, QB), :] = res.astype(bf16)

    def out_copy(p):
        o0 = p * (2 * QB)
        return pltpu.make_async_copy(x_v.at[pl.ds(o0, 2 * QB)], out_hbm.at[pl.ds(o0, 2 * QB)], o_sem)

    def pair_body(m0, masked, first):
        for j in range(2):
            m = m0 + j
            for g in range(4):
                if g < 3:
                    stage_a(m, g + 1, (g + 1) % 2, masked)
                elif j == 0:
                    stage_a(m + 1, 0, 0, masked)
                else:
                    stage_a(jnp.minimum(m + 1, M - 1), 0, 0, masked)
                stage_bc(m, g, g % 2, j)
            if not (first and j == 0):
                stage_d(m - 1, (j + 1) % 2)

    w_copies[1].wait()
    stage_a(0, 0, 0, True)
    pair_body(0, True, True)

    def loop_body(p, carry):
        pair_body(2 * p, False, False)
        out_copy(p - 1).start()
        return carry

    jax.lax.fori_loop(1, M // 2, loop_body, 0)
    stage_d(M - 1, 1)
    out_copy(M // 2 - 1).start()
    for p in range(M // 2):
        out_copy(p).wait()


@jax.jit
def pallas_parallel_sum__sliding_block__moe_arch_mod__prompt_kernel(
    A_x: jax.Array,
    A_wqkv: jax.Array,
    A_wo: jax.Array,
    B_x: jax.Array,
    B_w_r: jax.Array,
    B_w_gate: jax.Array,
    B_w_up: jax.Array,
    B_w_down: jax.Array,
):
    del B_x
    x = A_x.reshape(S, D)
    wr = B_w_r.reshape(1, D)
    bf16 = jnp.bfloat16
    f32 = jnp.float32
    any_spec = pl.BlockSpec(memory_space=pl.ANY)
    out = pl.pallas_call(
        _kernel,
        out_shape=jax.ShapeDtypeStruct((S, D), bf16),
        in_specs=[any_spec, any_spec, any_spec,
                  pl.BlockSpec(memory_space=pltpu.VMEM),
                  any_spec, any_spec, any_spec],
        out_specs=any_spec,
        scratch_shapes=[
            pltpu.VMEM((S, D), bf16),
            pltpu.VMEM((S, D), bf16),
            pltpu.VMEM((D, 3 * D), bf16),
            pltpu.VMEM((D, D), bf16),
            pltpu.VMEM((D, D), bf16),
            pltpu.VMEM((S, D), bf16),
            pltpu.VMEM((S + PAD, D), bf16),
            pltpu.VMEM((D, S + PAD), bf16),
            pltpu.VMEM((S, 1), f32),
            pltpu.VMEM((2 * QB, 8 * QB), f32),
            pltpu.VMEM((2 * QB, 8 * QB), f32),
            pltpu.VMEM((1, 8 * QB), f32),
            pltpu.VMEM((1, 8 * QB), f32),
            pltpu.VMEM((D, QB), f32),
            pltpu.VMEM((D, QB), f32),
            pltpu.VMEM((D, F), bf16),
            pltpu.VMEM((D, F), bf16),
            pltpu.VMEM((F, D), bf16),
            pltpu.VMEM((1, D), f32),
            pltpu.VMEM((1, 1), jnp.int32),
            pltpu.SemaphoreType.DMA((NCH,)),
            pltpu.SemaphoreType.DMA((5,)),
            pltpu.SemaphoreType.DMA,
        ],
        compiler_params=pltpu.CompilerParams(vmem_limit_bytes=96 * 1024 * 1024),
    )(x, A_wqkv, A_wo, wr, B_w_gate, B_w_up, B_w_down)
    return out.reshape(1, S, D)
```

```python
import jax
import jax.numpy as jnp
import jax.experimental.pallas as pl
import jax.experimental.pallas.tpu as pltpu

S = 2048
D = 512
H = 32
DH = 16
W = 256
F = 1376
NEG = -1e9
LOG2E = 1.4426950408889634
QSCALE = (DH ** -0.5) * LOG2E
R = 256
NCH = S // R
QB = 128
M = S // QB
PAD = 256

_NT = (((1,), (1,)), ((), ()))


def _bf(a):
    return a.astype(jnp.bfloat16).astype(jnp.float32)


def _kernel(x_hbm, wqkv_hbm, wo_hbm, wr_ref, wg_hbm, wu_hbm, wd_hbm, out_hbm,
            x_v, xn_v, wqkv_v, wvt_v, wo_v, q_v, k_v, vt_v, r_v,
            s_buf0, s_buf1, mx_buf0, mx_buf1, ot0, ot1,
            wg_v, wu_v, wd_v, moe_v, idx_v,
            x_sems, w_sems, o_sem):
    f32 = jnp.float32
    bf16 = jnp.bfloat16
    s_bufs = (s_buf0, s_buf1)
    mx_bufs = (mx_buf0, mx_buf1)
    ots = (ot0, ot1)

    def x_copy(c):
        return pltpu.make_async_copy(x_hbm.at[pl.ds(c * R, R)], x_v.at[pl.ds(c * R, R)], x_sems.at[c])

    w_copies = [
        pltpu.make_async_copy(wqkv_hbm, wqkv_v, w_sems.at[0]),
        pltpu.make_async_copy(wo_hbm, wo_v, w_sems.at[1]),
        pltpu.make_async_copy(wg_hbm, wg_v, w_sems.at[2]),
        pltpu.make_async_copy(wu_hbm, wu_v, w_sems.at[3]),
        pltpu.make_async_copy(wd_hbm, wd_v, w_sems.at[4]),
    ]
    x_copy(0).start()
    w_copies[0].start()
    for c in range(1, NCH):
        x_copy(c).start()
    for cp in w_copies[1:]:
        cp.start()

    k_v[0:PAD, :] = jnp.zeros((PAD, D), bf16)
    vt_v[:, 0:PAD] = jnp.zeros((D, PAD), bf16)

    w_copies[0].wait()
    wvt_v[...] = wqkv_v[:, 2 * D:3 * D].astype(f32).T.astype(bf16)

    wr = wr_ref[...].astype(f32)

    def phase0(c, carry):
        r0 = pl.multiple_of(c * R, R)
        x_copy(c).wait()
        xf = x_v[pl.ds(r0, R), :].astype(f32)
        mean = jnp.mean(xf, axis=-1, keepdims=True)
        var = jnp.mean(jnp.square(xf - mean), axis=-1, keepdims=True)
        dlt = _bf(xf - _bf(mean))
        den = _bf(jnp.sqrt(_bf(_bf(var) + 1e-5)))
        xn = (dlt / den).astype(bf16)
        xn_v[pl.ds(r0, R), :] = xn
        r_v[pl.ds(r0, R), :] = _bf(jnp.sum(xn.astype(f32) * wr, axis=-1, keepdims=True))
        qk = jnp.dot(xn, wqkv_v[:, 0:2 * D], preferred_element_type=f32)
        q_v[pl.ds(r0, R), :] = (qk[:, 0:D] * QSCALE).astype(bf16)
        k_v[pl.ds(PAD + r0, R), :] = qk[:, D:2 * D].astype(bf16)
        vt = jax.lax.dot_general(wvt_v[...], xn, _NT, preferred_element_type=f32)
        vt_v[:, pl.ds(PAD + r0, R)] = vt.astype(bf16)
        return carry

    jax.lax.fori_loop(0, NCH, phase0, 0)

    rr = r_v[...]
    rmax = jnp.max(rr, axis=0, keepdims=True)
    ids = jax.lax.broadcasted_iota(jnp.int32, (S, 1), 0)
    idx = jnp.min(jnp.where(rr == rmax, ids, S), axis=0, keepdims=True)
    idx_v[...] = idx

    def gather_row(c, acc):
        r0 = pl.multiple_of(c * R, R)
        rows = jax.lax.broadcasted_iota(jnp.int32, (R, D), 0) + r0
        xc = xn_v[pl.ds(r0, R), :].astype(f32)
        return acc + jnp.sum(jnp.where(rows == idx, xc, 0.0), axis=0, keepdims=True)

    x_sel = jax.lax.fori_loop(0, NCH, gather_row, jnp.zeros((1, D), f32))
    xs16 = jnp.broadcast_to(x_sel, (16, D)).astype(bf16)
    for cp in w_copies[2:]:
        cp.wait()
    gate = jax.lax.dot_general(xs16, wg_v[...], _NT, preferred_element_type=f32)
    up = jax.lax.dot_general(xs16, wu_v[...], _NT, preferred_element_type=f32)
    hmid = (gate * jax.nn.sigmoid(gate) * up).astype(bf16)
    y = jnp.dot(hmid, wd_v[...], preferred_element_type=f32)
    moe_v[...] = y[0:1, :] * jax.nn.sigmoid(rmax)

    lane = jax.lax.broadcasted_iota(jnp.int32, (QB, QB), 1)
    row = jax.lax.broadcasted_iota(jnp.int32, (QB, QB), 0)
    lane_head = lane // DH
    tri = row <= lane

    def stage_a(m, g, slot, masked):
        q0 = pl.multiple_of(m * QB, QB)
        gl = slice(g * 128, (g + 1) * 128)
        qs = q_v[pl.ds(q0, QB), gl]
        kf = k_v[pl.ds(q0, QB), gl]
        km = k_v[pl.ds(q0 + QB, QB), gl]
        kd = k_v[pl.ds(q0 + 2 * QB, QB), gl]
        parts = []
        for r in range(8):
            parts.append(kf[16 * r:16 * r + 16])
            parts.append(kd[16 * r:16 * r + 16])
        parts.append(km)
        ks = jnp.concatenate(parts, axis=0)
        qstack = jnp.concatenate(
            [jnp.where(lane_head == h, qs, jnp.zeros_like(qs)) for h in range(8)], axis=0)
        st = jax.lax.dot_general(ks, qstack, _NT, preferred_element_type=f32)
        for h in range(8):
            sl = slice(h * 128, (h + 1) * 128)
            mparts = []
            for r in range(8):
                far = st[32 * r:32 * r + 16, sl]
                diag = st[32 * r + 16:32 * r + 32, sl]
                if masked:
                    far = jnp.where(m >= 2, far, NEG)
                mparts.append(jnp.where(tri[16 * r:16 * r + 16], diag, far))
            mid = st[256:384, sl]
            if masked:
                mid = jnp.where(m >= 1, mid, NEG)
            sm = jnp.concatenate(mparts, axis=0)
            mx = jnp.maximum(jnp.max(sm, axis=0, keepdims=True), jnp.max(mid, axis=0, keepdims=True))
            s_bufs[slot][0:128, sl] = sm
            s_bufs[slot][128:256, sl] = mid
            mx_bufs[slot][:, sl] = mx

    def stage_bc(m, g, slot, oslot):
        q0 = pl.multiple_of(m * QB, QB)
        for h in range(8):
            sl = slice(h * 128, (h + 1) * 128)
            hh = g * 8 + h
            mx = mx_bufs[slot][:, sl]
            p_m = jnp.exp2(s_bufs[slot][0:128, sl] - mx)
            p_mid = jnp.exp2(s_bufs[slot][128:256, sl] - mx)
            l = jnp.sum(p_m, axis=0, keepdims=True) + jnp.sum(p_mid, axis=0, keepdims=True)
            zero = jnp.zeros_like(p_m)
            p = jnp.concatenate([jnp.where(tri, zero, p_m), p_mid, jnp.where(tri, p_m, zero)],
                                axis=0).astype(bf16)
            vt = vt_v[16 * hh:16 * hh + 16, pl.ds(q0, 3 * QB)]
            ot = jnp.dot(vt, p, preferred_element_type=f32)
            ots[oslot][16 * hh:16 * hh + 16, :] = ot / l

    def stage_d(m, oslot):
        q0 = pl.multiple_of(m * QB, QB)
        o = ots[oslot][...].T.astype(bf16)
        att = jnp.dot(o, wo_v[...], preferred_element_type=f32)
        rows = jax.lax.broadcasted_iota(jnp.int32, (QB, D), 0) + q0
        res = x_v[pl.ds(q0, QB), :].astype(f32) + xn_v[pl.ds(q0, QB), :].astype(f32) + att
        res = res + jnp.where(rows == idx_v[...], moe_v[...], 0.0)
        x_v[pl.ds(q0, QB), :] = res.astype(bf16)

    def out_copy(p):
        o0 = p * (2 * QB)
        return pltpu.make_async_copy(x_v.at[pl.ds(o0, 2 * QB)], out_hbm.at[pl.ds(o0, 2 * QB)], o_sem)

    def pair_body(m0, masked, first):
        for j in range(2):
            m = m0 + j
            for g in range(4):
                if g < 3:
                    stage_a(m, g + 1, (g + 1) % 2, masked)
                elif j == 0:
                    stage_a(m + 1, 0, 0, masked)
                else:
                    stage_a(jnp.minimum(m + 1, M - 1), 0, 0, masked)
                stage_bc(m, g, g % 2, j)
            if not (first and j == 0):
                stage_d(m - 1, (j + 1) % 2)

    w_copies[1].wait()
    stage_a(0, 0, 0, True)
    pair_body(0, True, True)

    def loop_body(p, carry):
        pair_body(2 * p, False, False)
        out_copy(p - 1).start()
        return carry

    jax.lax.fori_loop(1, M // 2, loop_body, 0)
    stage_d(M - 1, 1)
    out_copy(M // 2 - 1).start()
    for p in range(M // 2):
        out_copy(p).wait()


@jax.jit
def pallas_parallel_sum__sliding_block__moe_arch_mod__prompt_kernel(
    A_x: jax.Array,
    A_wqkv: jax.Array,
    A_wo: jax.Array,
    B_x: jax.Array,
    B_w_r: jax.Array,
    B_w_gate: jax.Array,
    B_w_up: jax.Array,
    B_w_down: jax.Array,
):
    del B_x
    x = A_x.reshape(S, D)
    wr = B_w_r.reshape(1, D)
    bf16 = jnp.bfloat16
    f32 = jnp.float32
    any_spec = pl.BlockSpec(memory_space=pltpu.MemorySpace.HBM)
    wgt = B_w_gate.T
    wut = B_w_up.T
    out = pl.pallas_call(
        _kernel,
        out_shape=jax.ShapeDtypeStruct((S, D), bf16),
        in_specs=[any_spec, any_spec, any_spec,
                  pl.BlockSpec(memory_space=pltpu.VMEM),
                  any_spec, any_spec, any_spec],
        out_specs=any_spec,
        scratch_shapes=[
            pltpu.VMEM((S, D), bf16),
            pltpu.VMEM((S, D), bf16),
            pltpu.VMEM((D, 3 * D), bf16),
            pltpu.VMEM((D, D), bf16),
            pltpu.VMEM((D, D), bf16),
            pltpu.VMEM((S, D), bf16),
            pltpu.VMEM((S + PAD, D), bf16),
            pltpu.VMEM((D, S + PAD), bf16),
            pltpu.VMEM((S, 1), f32),
            pltpu.VMEM((2 * QB, 8 * QB), f32),
            pltpu.VMEM((2 * QB, 8 * QB), f32),
            pltpu.VMEM((1, 8 * QB), f32),
            pltpu.VMEM((1, 8 * QB), f32),
            pltpu.VMEM((D, QB), f32),
            pltpu.VMEM((D, QB), f32),
            pltpu.VMEM((F, D), bf16),
            pltpu.VMEM((F, D), bf16),
            pltpu.VMEM((F, D), bf16),
            pltpu.VMEM((1, D), f32),
            pltpu.VMEM((1, 1), jnp.int32),
            pltpu.SemaphoreType.DMA((NCH,)),
            pltpu.SemaphoreType.DMA((5,)),
            pltpu.SemaphoreType.DMA,
        ],
        compiler_params=pltpu.CompilerParams(vmem_limit_bytes=96 * 1024 * 1024),
    )(x, A_wqkv, A_wo, wr, wgt, wut, B_w_down)
    return out.reshape(1, S, D)
```

```python
import jax
import jax.numpy as jnp
import jax.experimental.pallas as pl
import jax.experimental.pallas.tpu as pltpu

S = 2048
D = 512
H = 32
DH = 16
W = 256
F = 1376
NEG = -1e9
LOG2E = 1.4426950408889634
QSCALE = (DH ** -0.5) * LOG2E
R = 256
NCH = S // R
QB = 128
M = S // QB
PAD = 256

_NT = (((1,), (1,)), ((), ()))


def _bf(a):
    return a.astype(jnp.bfloat16).astype(jnp.float32)


def _kernel(x_hbm, wqkv_hbm, wo_hbm, wr_ref, wg_hbm, wu_hbm, wd_hbm, out_hbm,
            x_v, xn_v, wqkv_v, wvt_v, wo_v, q_v, k_v, vt_v, r_v,
            s_buf0, s_buf1, mx_buf0, mx_buf1, ot0, ot1,
            wg_v, wu_v, wd_v, moe_v, idx_v, xs0, xs1,
            x_sems, w_sems, o_sem):
    f32 = jnp.float32
    bf16 = jnp.bfloat16
    s_bufs = (s_buf0, s_buf1)
    mx_bufs = (mx_buf0, mx_buf1)
    ots = (ot0, ot1)

    def x_copy(c):
        return pltpu.make_async_copy(x_hbm.at[pl.ds(c * R, R)], x_v.at[pl.ds(c * R, R)], x_sems.at[c])

    w_copies = [
        pltpu.make_async_copy(wqkv_hbm.at[:, 0:D], wqkv_v.at[:, 0:D], w_sems.at[0]),
        pltpu.make_async_copy(wo_hbm, wo_v, w_sems.at[1]),
        pltpu.make_async_copy(wg_hbm, wg_v, w_sems.at[2]),
        pltpu.make_async_copy(wu_hbm, wu_v, w_sems.at[3]),
        pltpu.make_async_copy(wd_hbm, wd_v, w_sems.at[4]),
        pltpu.make_async_copy(wqkv_hbm.at[:, 2 * D:3 * D], wqkv_v.at[:, 2 * D:3 * D], w_sems.at[5]),
        pltpu.make_async_copy(wqkv_hbm.at[:, D:2 * D], wqkv_v.at[:, D:2 * D], w_sems.at[6]),
    ]
    x_copy(0).start()
    w_copies[0].start()
    w_copies[6].start()
    w_copies[5].start()
    for c in range(1, NCH):
        x_copy(c).start()
    for cp in w_copies[1:5]:
        cp.start()

    k_v[0:PAD, :] = jnp.zeros((PAD, D), bf16)
    vt_v[:, 0:PAD] = jnp.zeros((D, PAD), bf16)

    wr = wr_ref[...].astype(f32)

    xss = (xs0, xs1)

    def stage_ln(c, slot):
        r0 = pl.multiple_of(c * R, R)
        xf = x_v[pl.ds(r0, R), :].astype(f32)
        mean = jnp.mean(xf, axis=-1, keepdims=True)
        var = jnp.mean(jnp.square(xf - mean), axis=-1, keepdims=True)
        dlt = _bf(xf - _bf(mean))
        den = _bf(jnp.sqrt(_bf(_bf(var) + 1e-5)))
        xn = (dlt / den).astype(bf16)
        xn_v[pl.ds(r0, R), :] = xn
        xss[slot][...] = xn
        r_v[pl.ds(r0, R), :] = _bf(jnp.sum(xn.astype(f32) * wr, axis=-1, keepdims=True))

    def stage_qk(c, slot):
        r0 = pl.multiple_of(c * R, R)
        qk = jnp.dot(xss[slot][...], wqkv_v[:, 0:2 * D], preferred_element_type=f32)
        q_v[pl.ds(r0, R), :] = (qk[:, 0:D] * QSCALE).astype(bf16)
        k_v[pl.ds(PAD + r0, R), :] = qk[:, D:2 * D].astype(bf16)

    def stage_vt(c, slot):
        r0 = pl.multiple_of(c * R, R)
        vt = jax.lax.dot_general(wvt_v[...], xss[slot][...], _NT, preferred_element_type=f32)
        vt_v[:, pl.ds(PAD + r0, R)] = vt.astype(bf16)

    x_copy(0).wait()
    stage_ln(0, 0)
    w_copies[0].wait()
    x_copy(1).wait()
    q_v[0:R, :] = (jnp.dot(xss[0][...], wqkv_v[:, 0:D], preferred_element_type=f32) * QSCALE).astype(bf16)
    w_copies[6].wait()
    k_v[PAD:PAD + R, :] = jnp.dot(xss[0][...], wqkv_v[:, D:2 * D], preferred_element_type=f32).astype(bf16)
    stage_ln(1, 1)
    w_copies[5].wait()
    wvt_v[...] = wqkv_v[:, 2 * D:3 * D].astype(f32).T.astype(bf16)
    stage_vt(0, 0)

    def p0_body(p, carry):
        c = 2 * p + 1
        x_copy(c + 1).wait()
        x_copy(c + 2).wait()
        stage_ln(c + 1, 0)
        stage_qk(c, 1)
        stage_vt(c, 1)
        stage_ln(c + 2, 1)
        stage_qk(c + 1, 0)
        stage_vt(c + 1, 0)
        return carry

    jax.lax.fori_loop(0, (NCH - 2) // 2, p0_body, 0)

    for cp in w_copies[1:5]:
        cp.wait()

    def moe_branch():
        rr = r_v[...]
        rmax = jnp.max(rr, axis=0, keepdims=True)
        ids = jax.lax.broadcasted_iota(jnp.int32, (S, 1), 0)
        idx = jnp.min(jnp.where(rr == rmax, ids, S))
        idx_v[0] = idx
        base = pl.multiple_of((idx // 16) * 16, 16)
        x16 = xn_v[pl.ds(base, 16), :].astype(f32)
        rows16 = jax.lax.broadcasted_iota(jnp.int32, (16, D), 0) + base
        x_sel = jnp.sum(jnp.where(rows16 == idx, x16, 0.0), axis=0, keepdims=True)
        xs16 = jnp.broadcast_to(x_sel, (16, D)).astype(bf16)
        gate = jax.lax.dot_general(xs16, wg_v[...], _NT, preferred_element_type=f32)
        up = jax.lax.dot_general(xs16, wu_v[...], _NT, preferred_element_type=f32)
        hmid = (gate * jax.nn.sigmoid(gate) * up).astype(bf16)
        y = jnp.dot(hmid, wd_v[...], preferred_element_type=f32)
        moe_v[...] = y[0:1, :] * jax.nn.sigmoid(rmax)

    lane64 = jax.lax.broadcasted_iota(jnp.int32, (64, QB), 1)
    row64 = jax.lax.broadcasted_iota(jnp.int32, (64, QB), 0)
    lane_head64 = lane64 // DH
    tri64 = row64 <= (lane64 % 64)

    def stage_a(m, g, slot, masked, ts=(0, 1)):
        q0 = pl.multiple_of(m * QB, QB)
        gl = slice(g * 128, (g + 1) * 128)
        qs = q_v[pl.ds(q0, QB), gl]
        kf = k_v[pl.ds(q0, QB), gl]
        km = k_v[pl.ds(q0 + QB, QB), gl]
        kd = k_v[pl.ds(q0 + 2 * QB, QB), gl]
        q_lo, q_hi = qs[0:64], qs[64:128]
        zq = jnp.zeros_like(q_lo)
        lh = lane_head64
        for t in ts:
            o = 64 * t
            parts = []
            for r in range(4):
                parts.append(kf[o + 16 * r:o + 16 * r + 16])
                parts.append(kd[o + 16 * r:o + 16 * r + 16])
            parts.append(kf[64:128] if t == 0 else kd[0:64])
            parts.append(km)
            ks = jnp.concatenate(parts, axis=0)
            wparts = []
            for u in range(4):
                if t == 0:
                    wparts.append(jnp.where(lh == 2 * u, q_lo, zq))
                    wparts.append(jnp.where(lh == 2 * u + 1, q_lo, zq))
                else:
                    wparts.append(jnp.where(lh == 2 * u + 1, q_hi, zq))
                    wparts.append(jnp.where(lh == 2 * u, q_hi, zq))
            qstack = jnp.concatenate(wparts, axis=0)
            st = jax.lax.dot_general(ks, qstack, _NT, preferred_element_type=f32)
            for u in range(4):
                sl = slice(u * 128, (u + 1) * 128)
                cl = slice((4 * t + u) * 128, (4 * t + u + 1) * 128)
                mparts = []
                for r in range(4):
                    far = st[32 * r:32 * r + 16, sl]
                    diag = st[32 * r + 16:32 * r + 32, sl]
                    if masked:
                        far = jnp.where(m >= 2, far, NEG)
                    mparts.append(jnp.where(tri64[16 * r:16 * r + 16], diag, far))
                full = st[128:192, sl]
                if masked and t == 0:
                    full = jnp.where(m >= 2, full, NEG)
                mid = st[192:320, sl]
                if masked:
                    mid = jnp.where(m >= 1, mid, NEG)
                sm = jnp.concatenate(mparts + [full], axis=0)
                mx = jnp.maximum(jnp.max(sm, axis=0, keepdims=True), jnp.max(mid, axis=0, keepdims=True))
                s_bufs[slot][0:128, cl] = sm
                s_bufs[slot][128:256, cl] = mid
                mx_bufs[slot][:, cl] = mx

    def stage_bc(m, g, slot, oslot, ts=(0, 1)):
        q0 = pl.multiple_of(m * QB, QB)
        z64 = jnp.zeros((64, 128), f32)
        for t in ts:
            lsl = slice(64 * t, 64 * t + 64)
            for u in range(4):
                hh = g * 8 + 2 * u
                vt2 = vt_v[16 * hh:16 * hh + 32, pl.ds(q0, 3 * QB)]
                cl = slice((4 * t + u) * 128, (4 * t + u + 1) * 128)
                mx = mx_bufs[slot][:, cl]
                p_top = jnp.exp2(s_bufs[slot][0:128, cl] - mx)
                p_mid = jnp.exp2(s_bufs[slot][128:256, cl] - mx)
                l = jnp.sum(p_top, axis=0, keepdims=True) + jnp.sum(p_mid, axis=0, keepdims=True)
                pm, pf = p_top[0:64], p_top[64:128]
                p_far = jnp.where(tri64, 0.0, pm)
                p_diag = jnp.where(tri64, pm, 0.0)
                if t == 0:
                    pieces = [p_far, pf, p_mid, p_diag, z64]
                else:
                    pieces = [z64, p_far, p_mid, pf, p_diag]
                p = jnp.concatenate(pieces, axis=0).astype(bf16)
                o = jnp.dot(vt2, p, preferred_element_type=f32) / l
                ots[oslot][16 * hh:16 * hh + 16, lsl] = o[0:16, lsl]
                ots[oslot][16 * hh + 16:16 * hh + 32, lsl] = pltpu.roll(o[16:32], 64, 1)[:, lsl]

    def stage_d(m, oslot):
        q0 = pl.multiple_of(m * QB, QB)
        o = ots[oslot][...].T.astype(bf16)
        att = jnp.dot(o, wo_v[...], preferred_element_type=f32)
        rows = jax.lax.broadcasted_iota(jnp.int32, (QB, D), 0) + q0
        res = x_v[pl.ds(q0, QB), :].astype(f32) + xn_v[pl.ds(q0, QB), :].astype(f32) + att
        res = res + jnp.where(rows == idx_v[0], moe_v[...], 0.0)
        x_v[pl.ds(q0, QB), :] = res.astype(bf16)

    def out_copy(p):
        o0 = p * (2 * QB)
        return pltpu.make_async_copy(x_v.at[pl.ds(o0, 2 * QB)], out_hbm.at[pl.ds(o0, 2 * QB)], o_sem)

    def pair_body(m0, masked, first, last=False):
        for j in range(2):
            m = m0 + j
            for g in range(4):
                for t in range(2):
                    if g < 3:
                        stage_a(m, g + 1, (g + 1) % 2, masked, (t,))
                    elif j == 0:
                        stage_a(m + 1, 0, 0, masked, (t,))
                    elif not last:
                        stage_a(m + 1, 0, 0, masked, (t,))
                    stage_bc(m, g, g % 2, j, (t,))
            if not (first and j == 0):
                stage_d(m - 1, (j + 1) % 2)

    stage_qk(NCH - 1, 1)
    stage_vt(NCH - 1, 1)
    moe_branch()
    stage_a(0, 0, 0, True)
    pair_body(0, True, True)

    def loop_body(p, carry):
        pair_body(2 * p, False, False)
        out_copy(p - 1).start()
        return carry

    jax.lax.fori_loop(1, M // 2 - 1, loop_body, 0)
    pair_body(M - 2, False, False, last=True)
    out_copy(M // 2 - 2).start()
    stage_d(M - 1, 1)
    out_copy(M // 2 - 1).start()
    for p in range(M // 2):
        out_copy(p).wait()


@jax.jit
def pallas_parallel_sum__sliding_block__moe_arch_mod__prompt_kernel(
    A_x: jax.Array,
    A_wqkv: jax.Array,
    A_wo: jax.Array,
    B_x: jax.Array,
    B_w_r: jax.Array,
    B_w_gate: jax.Array,
    B_w_up: jax.Array,
    B_w_down: jax.Array,
):
    del B_x
    x = A_x.reshape(S, D)
    wr = B_w_r.reshape(1, D)
    bf16 = jnp.bfloat16
    f32 = jnp.float32
    any_spec = pl.BlockSpec(memory_space=pltpu.MemorySpace.HBM)
    wgt = B_w_gate.T
    wut = B_w_up.T
    out = pl.pallas_call(
        _kernel,
        out_shape=jax.ShapeDtypeStruct((S, D), bf16),
        in_specs=[any_spec, any_spec, any_spec,
                  pl.BlockSpec(memory_space=pltpu.VMEM),
                  any_spec, any_spec, any_spec],
        out_specs=any_spec,
        scratch_shapes=[
            pltpu.VMEM((S, D), bf16),
            pltpu.VMEM((S, D), bf16),
            pltpu.VMEM((D, 3 * D), bf16),
            pltpu.VMEM((D, D), bf16),
            pltpu.VMEM((D, D), bf16),
            pltpu.VMEM((S, D), bf16),
            pltpu.VMEM((S + PAD, D), bf16),
            pltpu.VMEM((D, S + PAD), bf16),
            pltpu.VMEM((S, 1), f32),
            pltpu.VMEM((2 * QB, 8 * QB), f32),
            pltpu.VMEM((2 * QB, 8 * QB), f32),
            pltpu.VMEM((1, 8 * QB), f32),
            pltpu.VMEM((1, 8 * QB), f32),
            pltpu.VMEM((D, QB), f32),
            pltpu.VMEM((D, QB), f32),
            pltpu.VMEM((F, D), bf16),
            pltpu.VMEM((F, D), bf16),
            pltpu.VMEM((F, D), bf16),
            pltpu.VMEM((1, D), f32),
            pltpu.SMEM((1,), jnp.int32),
            pltpu.VMEM((R, D), bf16),
            pltpu.VMEM((R, D), bf16),
            pltpu.SemaphoreType.DMA((NCH,)),
            pltpu.SemaphoreType.DMA((7,)),
            pltpu.SemaphoreType.DMA,
        ],
        compiler_params=pltpu.CompilerParams(vmem_limit_bytes=96 * 1024 * 1024),
    )(x, A_wqkv, A_wo, wr, wgt, wut, B_w_down)
    return out.reshape(1, S, D)
```
